```python
import os as _os
_os.environ.setdefault("JAX_PLATFORMS", "cpu")
import jax
import jax.numpy as jnp

def _softmax(x, axis=-1):
    return jax.nn.softmax(x, axis=axis)
def _gelu(x):
    return jax.nn.gelu(x, approximate=True)
def _silu(x):
    return jax.nn.silu(x)
def _sigmoid(x):
    return jax.nn.sigmoid(x)
def _layernorm(x, axis=-1, eps=1e-5):
    m = jnp.mean(x, axis=axis, keepdims=True)
    v = jnp.var(x, axis=axis, keepdims=True)
    return (x - m) / jnp.sqrt(v + eps)
def _scatter_add(tgt, idx, src, axis=0):
    return tgt.at[idx].add(src)
def _segment_sum(src, seg, n):
    return jax.ops.segment_sum(src, seg, n)
class _Rng:
    def __init__(self, key):
        self._k = key
    def _next(self):
        self._k, sub = jax.random.split(self._k)
        return sub
    def normal(self, shape):
        return jax.random.normal(self._next(), shape, dtype=jnp.bfloat16)
    def randint(self, lo, hi, shape):
        return jax.random.randint(self._next(), shape, lo, hi, dtype=jnp.int32)
    def uniform(self, shape, lo=0.0, hi=1.0):
        return jax.random.uniform(self._next(), shape, jnp.bfloat16, lo, hi)
    def permutation(self, n):
        return jax.random.permutation(self._next(), n)


kernel_name = 'standalone__gqa_softmax__near_ridge'

def setup_inputs():
    _rng = _Rng(jax.random.key(int.from_bytes(__import__("os").urandom(4), "little")))
    _w = (lambda a: (lambda t: t.astype(jnp.bfloat16) if jnp.issubdtype(t.dtype, jnp.floating) else t)(jnp.asarray(a)))
    B, Hq, Hkv, Sq, Sk, D = 8, 32, 8, 112, 2048, 128
    return {
        "q": _w((lambda *s: _rng.normal(s) * 0.4)(B, Hq, Sq, D)),
        "k": _w((lambda *s: _rng.normal(s) * 0.4)(B, Hkv, Sk, D)),
        "v": _w((lambda *s: _rng.normal(s) * 0.05)(B, Hkv, Sk, D)),
    }

def reference(q, k, v):
    B, Hq, Sq, D = q.shape
    Hkv = k.shape[1]
    rep = Hq // Hkv
    k = jnp.repeat(k, rep, axis=1)
    v = jnp.repeat(v, rep, axis=1)
    scale = D ** -0.5
    scores = jnp.einsum("bhqd,bhkd->bhqk", q, k) * scale
    p = _softmax(scores, axis=-1)
    return jnp.einsum("bhqk,bhkd->bhqd", p, v)
```

```python
import functools
import jax, jax.numpy as jnp
from jax import lax
from jax.experimental import pallas as pl
from jax.experimental.pallas import tpu as pltpu

LOG2E = 1.4426950408889634
LP = {"XLA_TPU_FORCE_LP_LLO_SCHEDULER": True}

def qk(q, k):
    return lax.dot_general(q, k, (((1,), (1,)), ((), ())), preferred_element_type=jnp.float32)

def lanemax(s):
    r = s[:, :128]
    for t in range(1, s.shape[1] // 128):
        r = jnp.maximum(r, s[:, t*128:(t+1)*128])
    return r

def lanesum(s):
    r = s[:, :128]
    for t in range(1, s.shape[1] // 128):
        r = r + s[:, t*128:(t+1)*128]
    return r

def make_m(U, pattern, KB=512, flags=None, qmode="jit", fmode="newton", N1=3, nit=None, peel=True):
    NS = 3 if (U % 3 == 0) else 2
    pats = pattern if isinstance(pattern, (list, tuple)) else [pattern] * U
    def kern(q_hbm, k_hbm, v_hbm, o_hbm, qb, kb, vb, ob, qp, kp, vp, op, *rest):
        S = rest[:NS]; M = rest[NS:2*NS]
        sem_in, sem_out, semp, sempo = rest[2*NS:]
        G, R, D = q_hbm.shape
        Sk = k_hbm.shape[1]
        NB = Sk // KB
        c = D ** -0.5 * LOG2E
        assert (G - 1 - N1) % U == 0
        NIT = nit or (G - 1 - N1) // U

        def run(toks, qf, k_ref, sa, ma, sb, mb, v_ref, o_ref):
            doA = qf is not None; doB = sb is not None
            st = {}
            for t in toks.split():
                if t[0] == 'A' and doA:
                    j = int(t[1:])
                    if qmode == "once":
                        if 'q' not in st:
                            st['q'] = (qf(0)[...].astype(jnp.float32) * c).astype(jnp.bfloat16)
                        q = st['q']
                    elif qmode == "jit":
                        q = (qf(j)[...].astype(jnp.float32) * c).astype(jnp.bfloat16)
                    else:
                        q = qf(j)[...]
                    s = qk(q, k_ref[j*KB:(j+1)*KB, :])
                    sa[:, j*KB:(j+1)*KB] = s
                    pm = lanemax(s)
                    st['pm'] = pm if 'pm' not in st else jnp.maximum(st['pm'], pm)
                    if j == NB - 1:
                        ma[...] = st['pm']
                elif t == 'M' and doB:
                    st['m'] = jnp.broadcast_to(jnp.max(mb[...], axis=-1, keepdims=True), (R, 128))
                elif t[0] == 'B' and doB:
                    j = int(t[1:])
                    s = sb[:, j*KB:(j+1)*KB]
                    x = s - jnp.tile(st['m'], (1, KB // 128))
                    if qmode == "late":
                        x = x * c
                    p = jnp.exp2(x)
                    ls = lanesum(p)
                    st['l'] = ls if 'l' not in st else st['l'] + ls
                    o = jnp.dot(p.astype(jnp.bfloat16), v_ref[j*KB:(j+1)*KB, :], preferred_element_type=jnp.float32)
                    st['o'] = o if 'o' not in st else st['o'] + o
                elif t == 'F' and doB:
                    l = jnp.sum(st['l'], axis=-1, keepdims=True)
                    if fmode == "div":
                        o_ref[...] = (st['o'] / l).astype(o_ref.dtype)
                    else:
                        r = pl.reciprocal(l, approx=True)
                        r = r * (2.0 - l * r)
                        o_ref[...] = (st['o'] * r).astype(o_ref.dtype)

        def in_copies(it, slot):
            h = N1 + it * U
            return [pltpu.make_async_copy(v_hbm.at[pl.ds(h, U)], vb.at[slot], sem_in.at[slot, 0]),
                    pltpu.make_async_copy(k_hbm.at[pl.ds(h + 1, U)], kb.at[slot], sem_in.at[slot, 1]),
                    pltpu.make_async_copy(q_hbm.at[pl.ds(h + 1, U)], qb.at[slot], sem_in.at[slot, 2])]
        def out_copy(it, slot):
            return pltpu.make_async_copy(ob.at[slot], o_hbm.at[pl.ds(N1 + it * U, U)], sem_out.at[slot])
        def pk(h): return pltpu.make_async_copy(k_hbm.at[h], kp.at[h], semp.at[h, 0])
        def pq(h): return pltpu.make_async_copy(q_hbm.at[h], qp.at[h], semp.at[h, 1])
        def pv(h): return pltpu.make_async_copy(v_hbm.at[h], vp.at[h], semp.at[h, 2])
        def po(h): return pltpu.make_async_copy(op.at[h], o_hbm.at[h], sempo.at[h])
        last_v = pltpu.make_async_copy(v_hbm.at[G - 1], vp.at[N1], semp.at[N1, 2])
        last_o = pltpu.make_async_copy(op.at[N1], o_hbm.at[G - 1], sempo.at[N1])

        pq(0).start(); pk(0).start()
        if N1 > 0:
            pq(1).start(); pk(1).start(); pv(0).start()
        else:
            for x in in_copies(0, 0): x.start()
        pq(0).wait(); pk(0).wait()
        run(pats[0], lambda j: qp.at[0], kp.at[0], S[0].at[0], M[0].at[0], None, None, None, None)
        for h in range(N1):
            pq(h + 1).wait(); pk(h + 1).wait(); pv(h).wait()
            if h + 1 < N1:
                pq(h + 2).start(); pk(h + 2).start(); pv(h + 1).start()
            else:
                for x in in_copies(0, 0): x.start()
            z = pl.program_id(0) if False else 0
            run(pats[0], lambda j, h=h: qp.at[h + 1], kp.at[h + 1], S[(h + 1) % NS].at[0], M[(h + 1) % NS].at[0],
                S[h % NS].at[0], M[h % NS].at[0], vp.at[h], op.at[h])
            po(h).start()
        for x in in_copies(0, 0): x.wait()
        for x in in_copies(1, 1): x.start()
        last_v.start()

        def body(it, carry):
            slot = it & 1
            z1 = it >> 12; z2 = (it + 1) >> 12
            @pl.when(it >= 2)
            def _():
                out_copy(it - 2, slot).wait()
            @pl.when(it >= 1)
            def _():
                for x in in_copies(it, slot): x.wait()
            for u in range(U):
                qf = lambda j, u=u: qb.at[slot, u + ((it + j) >> 12)]
                a = (N1 + u + 1) % NS; b = (N1 + u) % NS
                run(pats[u], qf, kb.at[slot, u], S[a].at[z1], M[a].at[z1], S[b].at[z2], M[b].at[z2], vb.at[slot, u], ob.at[slot, u])
            out_copy(it, slot).start()
            @pl.when(it + 2 < NIT)
            def _():
                for x in in_copies(it + 2, slot): x.start()
            return carry
        lax.fori_loop(0, NIT, body, 0)
        last_v.wait()
        run(pats[0], None, None, None, None, S[(G - 1) % NS].at[0], M[(G - 1) % NS].at[0], vp.at[N1], op.at[N1])
        last_o.start()
        out_copy(NIT - 2, (NIT - 2) % 2).wait()
        out_copy(NIT - 1, (NIT - 1) % 2).wait()
        for h in range(N1): po(h).wait()
        last_o.wait()

    def f(q, k, v):
        Bn, Hq, Sq, D = q.shape
        Hkv, Sk = k.shape[1], k.shape[2]
        G = Bn * Hkv; R = (Hq // Hkv) * Sq
        q2 = q.reshape(G, R, D); k2 = k.reshape(G, Sk, D); v2 = v.reshape(G, Sk, D)
        anyspec = pl.BlockSpec(memory_space=pl.ANY)
        sm = [pltpu.VMEM((1, R, Sk), jnp.float32)] * NS + [pltpu.VMEM((1, R, 128), jnp.float32)] * NS
        dt = q.dtype
        o = pl.pallas_call(
            kern, grid=(),
            in_specs=[anyspec] * 3, out_specs=anyspec,
            out_shape=jax.ShapeDtypeStruct((G, R, D), dt),
            scratch_shapes=[pltpu.VMEM((2, U, R, D), dt), pltpu.VMEM((2, U, Sk, D), dt),
                            pltpu.VMEM((2, U, Sk, D), dt), pltpu.VMEM((2, U, R, D), dt),
                            pltpu.VMEM((N1 + 1, R, D), dt), pltpu.VMEM((N1 + 1, Sk, D), dt),
                            pltpu.VMEM((N1 + 1, Sk, D), dt), pltpu.VMEM((N1 + 1, R, D), dt)]
                           + sm
                           + [pltpu.SemaphoreType.DMA((2, 3)), pltpu.SemaphoreType.DMA((2,)),
                              pltpu.SemaphoreType.DMA((N1 + 1, 3)), pltpu.SemaphoreType.DMA((N1 + 1,))],
            compiler_params=pltpu.CompilerParams(vmem_limit_bytes=100*2**20, flags=flags, disable_bounds_checks=True),
        )(q2, k2, v2)
        return o.reshape(Bn, Hq, Sq, D)
    return f

O4 = "M A0 A1 B0 B1 B2 B3 F A2 A3"
O3 = "M A0 B0 A1 B1 A2 B2 B3 F A3"
O1 = "M A0 B0 A1 B1 A2 B2 A3 B3 F"
O6 = "M A0 A1 A2 B0 B1 B2 B3 F A3"
O5 = "M A0 B0 B1 B2 B3 F A1 A2 A3"

_impl = make_m(3, O6, 512, LP, "jit", "newton")


@jax.jit
def pallas_standalone__gqa_softmax__near_ridge_kernel(q, k, v):
    return _impl(q, k, v)
```

```python
import functools
import jax, jax.numpy as jnp
from jax import lax
from jax.experimental import pallas as pl
from jax.experimental.pallas import tpu as pltpu

LOG2E = 1.4426950408889634
LP = {"XLA_TPU_FORCE_LP_LLO_SCHEDULER": True}

def qk(q, k):
    return lax.dot_general(q, k, (((1,), (1,)), ((), ())), preferred_element_type=jnp.float32)

def lanemax(s):
    r = s[:, :128]
    for t in range(1, s.shape[1] // 128):
        r = jnp.maximum(r, s[:, t*128:(t+1)*128])
    return r

def lanesum(s):
    r = s[:, :128]
    for t in range(1, s.shape[1] // 128):
        r = r + s[:, t*128:(t+1)*128]
    return r

def make_m(U, pattern, KB=512, flags=None, qmode="jit", fmode="newton", N1=3, nit=None, STG=None, split0=False, vsplit=0, nob=True):
    NS = 3 if (U % 3 == 0) else 2
    pats = pattern if isinstance(pattern, (list, tuple)) else [pattern] * U
    def kern(q_hbm, k_hbm, v_hbm, o_hbm, qb, kb, vb, ob, qp, kp, vp, op, *rest):
        S = rest[:NS]; M = rest[NS:2*NS]
        sem_in, sem_out, semp, sempo, sem_s0, semk0 = rest[2*NS:]
        G, R, D = q_hbm.shape
        Sk = k_hbm.shape[1]
        NB = Sk // KB
        c = D ** -0.5 * LOG2E
        assert (G - 1 - N1) % U == 0
        NIT = nit or (G - 1 - N1) // U

        def run(toks, qf, k_ref, sa, ma, sb, mb, v_ref, o_ref, st=None):
            doA = qf is not None; doB = sb is not None
            st = {} if st is None else st
            for t in toks.split():
                if t[0] == 'A' and doA:
                    j = int(t[1:])
                    if qmode == "once":
                        if 'q' not in st:
                            st['q'] = (qf(0)[...].astype(jnp.float32) * c).astype(jnp.bfloat16)
                        q = st['q']
                    elif qmode == "jit":
                        q = (qf(j)[...].astype(jnp.float32) * c).astype(jnp.bfloat16)
                    else:
                        q = qf(j)[...]
                    s = qk(q, k_ref[j*KB:(j+1)*KB, :])
                    sa[:, j*KB:(j+1)*KB] = s
                    pm = lanemax(s)
                    st['pm'] = pm if 'pm' not in st else jnp.maximum(st['pm'], pm)
                    if j == NB - 1:
                        ma[...] = st['pm']
                elif t == 'M' and doB:
                    st['m'] = jnp.broadcast_to(jnp.max(mb[...], axis=-1, keepdims=True), (R, 128))
                elif t[0] == 'B' and doB:
                    j = int(t[1:])
                    s = sb[:, j*KB:(j+1)*KB]
                    x = s - jnp.tile(st['m'], (1, KB // 128))
                    if qmode == "late":
                        x = x * c
                    p = jnp.exp2(x)
                    ls = lanesum(p)
                    st['l'] = ls if 'l' not in st else st['l'] + ls
                    o = jnp.dot(p.astype(jnp.bfloat16), v_ref[j*KB:(j+1)*KB, :], preferred_element_type=jnp.float32)
                    st['o'] = o if 'o' not in st else st['o'] + o
                elif t == 'F' and doB:
                    l = jnp.sum(st['l'], axis=-1, keepdims=True)
                    if fmode == "div":
                        o_ref[...] = (st['o'] / l).astype(o_ref.dtype)
                    else:
                        r = pl.reciprocal(l, approx=True)
                        r = r * (2.0 - l * r)
                        o_ref[...] = (st['o'] * r).astype(o_ref.dtype)

        def in_copies(it, slot):
            h = N1 + it * U
            return [pltpu.make_async_copy(v_hbm.at[pl.ds(h, U)], vb.at[slot], sem_in.at[slot, 0]),
                    pltpu.make_async_copy(k_hbm.at[pl.ds(h + 1, U)], kb.at[slot], sem_in.at[slot, 1]),
                    pltpu.make_async_copy(q_hbm.at[pl.ds(h + 1, U)], qb.at[slot], sem_in.at[slot, 2])]
        def out_copy(it, slot):
            return pltpu.make_async_copy(ob.at[slot], o_hbm.at[pl.ds(N1 + it * U, U)], sem_out.at[slot])
        def pk(h): return pltpu.make_async_copy(k_hbm.at[h], kp.at[h], semp.at[h, 0])
        def pq(h): return pltpu.make_async_copy(q_hbm.at[h], qp.at[h], semp.at[h, 1])
        def pv(h): return pltpu.make_async_copy(v_hbm.at[h], vp.at[h], semp.at[h, 2])
        def po(h): return pltpu.make_async_copy(op.at[h], o_hbm.at[h], sempo.at[h])
        last_v = pltpu.make_async_copy(v_hbm.at[G - 1], vp.at[N1], semp.at[N1, 2])
        last_o = pltpu.make_async_copy(op.at[N1], o_hbm.at[G - 1], sempo.at[N1])

        def s0(kind, u):
            h = N1 + u
            if kind == 'k': return pltpu.make_async_copy(k_hbm.at[h + 1], kb.at[0, u], sem_s0.at[0, u])
            if kind == 'v': return pltpu.make_async_copy(v_hbm.at[h], vb.at[0, u], sem_s0.at[1, u])
            if kind == 'q': return pltpu.make_async_copy(q_hbm.at[h + 1], qb.at[0, u], sem_s0.at[2, u])
        def issue(stage):
            for piece in STG.get(stage, "").split():
                s0(piece[0], int(piece[1:])).start()
        kc = [pltpu.make_async_copy(k_hbm.at[0, pl.ds(j * (Sk // 2), Sk // 2)], kp.at[0, pl.ds(j * (Sk // 2), Sk // 2)], semk0.at[j]) for j in range(2)]
        pq(0).start()
        if split0:
            kc[0].start(); kc[1].start()
        else:
            pk(0).start()
        for h in range(N1):
            pq(h + 1).start(); pk(h + 1).start(); pv(h).start()
        issue('t0')
        pq(0).wait()
        if split0:
            kc[0].wait()
        else:
            pk(0).wait()
        issue('a0')
        if split0:
            st0 = {}
            run("A0 A1", lambda j: qp.at[0], kp.at[0], S[0].at[0], M[0].at[0], None, None, None, None, st0)
            kc[1].wait()
            run("A2 A3", lambda j: qp.at[0], kp.at[0], S[0].at[0], M[0].at[0], None, None, None, None, st0)
        else:
            run(pats[0], lambda j: qp.at[0], kp.at[0], S[0].at[0], M[0].at[0], None, None, None, None)
        for h in range(N1):
            pq(h + 1).wait(); pk(h + 1).wait()
            args = (lambda j, h=h: qp.at[h + 1], kp.at[h + 1], S[(h + 1) % NS].at[0], M[(h + 1) % NS].at[0],
                    S[h % NS].at[0], M[h % NS].at[0], vp.at[h], op.at[h])
            if h < vsplit:
                sth = {}
                run("M A0 A1 A2", *args, sth)
                pv(h).wait()
                issue(f'p{h}')
                run("B0 B1 B2 B3 F A3", *args, sth)
            else:
                pv(h).wait()
                issue(f'p{h}')
                run(pats[0], *args)
            po(h).start()
        for kind in 'kvq':
            for u in range(U): s0(kind, u).wait()
        for x in in_copies(1, 1): x.start()
        last_v.start()

        def body(it, carry):
            slot = it & 1
            z1 = it >> 12; z2 = (it + 1) >> 12
            @pl.when(it >= 2)
            def _():
                out_copy(it - 2, slot).wait()
            @pl.when(it >= 1)
            def _():
                for x in in_copies(it, slot): x.wait()
            for u in range(U):
                qf = lambda j, u=u: qb.at[slot, u + ((it + j) >> 12)]
                a = (N1 + u + 1) % NS; b = (N1 + u) % NS
                run(pats[u], qf, kb.at[slot, u], S[a].at[z1], M[a].at[z1], S[b].at[z2], M[b].at[z2], vb.at[slot, u], ob.at[slot, u])
            out_copy(it, slot).start()
            @pl.when(it + 2 < NIT)
            def _():
                for x in in_copies(it + 2, slot): x.start()
            return carry
        lax.fori_loop(0, NIT, body, 0)
        last_v.wait()
        run(pats[0], None, None, None, None, S[(G - 1) % NS].at[0], M[(G - 1) % NS].at[0], vp.at[N1], op.at[N1])
        last_o.start()
        out_copy(NIT - 2, (NIT - 2) % 2).wait()
        out_copy(NIT - 1, (NIT - 1) % 2).wait()
        for h in range(N1): po(h).wait()
        last_o.wait()

    def f(q, k, v):
        Bn, Hq, Sq, D = q.shape
        Hkv, Sk = k.shape[1], k.shape[2]
        G = Bn * Hkv; R = (Hq // Hkv) * Sq
        q2 = q.reshape(G, R, D); k2 = k.reshape(G, Sk, D); v2 = v.reshape(G, Sk, D)
        anyspec = pl.BlockSpec(memory_space=pl.ANY)
        sm = [pltpu.VMEM((1, R, Sk), jnp.float32)] * NS + [pltpu.VMEM((1, R, 128), jnp.float32)] * NS
        dt = q.dtype
        o = pl.pallas_call(
            kern, grid=(),
            in_specs=[anyspec] * 3, out_specs=anyspec,
            out_shape=jax.ShapeDtypeStruct((G, R, D), dt),
            scratch_shapes=[pltpu.VMEM((2, U, R, D), dt), pltpu.VMEM((2, U, Sk, D), dt),
                            pltpu.VMEM((2, U, Sk, D), dt), pltpu.VMEM((2, U, R, D), dt),
                            pltpu.VMEM((N1 + 1, R, D), dt), pltpu.VMEM((N1 + 1, Sk, D), dt),
                            pltpu.VMEM((N1 + 1, Sk, D), dt), pltpu.VMEM((N1 + 1, R, D), dt)]
                           + sm
                           + [pltpu.SemaphoreType.DMA((2, 3)), pltpu.SemaphoreType.DMA((2,)),
                              pltpu.SemaphoreType.DMA((N1 + 1, 3)), pltpu.SemaphoreType.DMA((N1 + 1,)), pltpu.SemaphoreType.DMA((3, U)), pltpu.SemaphoreType.DMA((2,))],
            compiler_params=pltpu.CompilerParams(vmem_limit_bytes=100*2**20, flags=flags, disable_bounds_checks=nob),
        )(q2, k2, v2)
        return o.reshape(Bn, Hq, Sq, D)
    return f

O4 = "M A0 A1 B0 B1 B2 B3 F A2 A3"
O3 = "M A0 B0 A1 B1 A2 B2 B3 F A3"
O1 = "M A0 B0 A1 B1 A2 B2 A3 B3 F"
O6 = "M A0 A1 A2 B0 B1 B2 B3 F A3"
O5 = "M A0 B0 B1 B2 B3 F A1 A2 A3"

_impl = make_m(4, O6, 512, LP, "jit", "newton", N1=7, STG={"p2": " ".join(f"q{u} k{u} v{u}" for u in range(4))}, split0=True, vsplit=1, nob=False)


@jax.jit
def pallas_standalone__gqa_softmax__near_ridge_kernel(q, k, v):
    return _impl(q, k, v)
```

```python
import jax
import jax.numpy as jnp
from jax import lax
from jax.experimental import pallas as pl
from jax.experimental.pallas import tpu as pltpu

LOG2E = 1.4426950408889634
U = 4
N1 = 7
NS = 2
KB = 512
LANES = 128


def _lane_reduce(op, s):
    r = s[:, :LANES]
    for t in range(1, s.shape[1] // LANES):
        r = op(r, s[:, t * LANES:(t + 1) * LANES])
    return r


def _kernel(q_hbm, k_hbm, v_hbm, o_hbm, qb, kb, vb, ob, qp, kp, vp, op,
            s0, s1, m0, m1, sem_in, sem_out, semp, sempo, sem_s0, semk0):
    S, M = (s0, s1), (m0, m1)
    G, R, D = q_hbm.shape
    Sk = k_hbm.shape[1]
    NB = Sk // KB
    c = D ** -0.5 * LOG2E
    assert NB == 4 and (G - 1 - N1) % U == 0
    NIT = (G - 1 - N1) // U

    def run(toks, qf, k_ref, sa, ma, sb, mb, v_ref, o_ref, st=None):
        st = {} if st is None else st
        for t in toks.split():
            if t[0] == 'A' and qf is not None:
                j = int(t[1:])
                q = (qf(j)[...].astype(jnp.float32) * c).astype(jnp.bfloat16)
                s = lax.dot_general(q, k_ref[j * KB:(j + 1) * KB, :], (((1,), (1,)), ((), ())),
                                    preferred_element_type=jnp.float32)
                sa[:, j * KB:(j + 1) * KB] = s
                pm = _lane_reduce(jnp.maximum, s)
                st['pm'] = pm if 'pm' not in st else jnp.maximum(st['pm'], pm)
                if j == NB - 1:
                    ma[...] = st['pm']
            elif t == 'M' and sb is not None:
                st['m'] = jnp.broadcast_to(jnp.max(mb[...], axis=-1, keepdims=True), (R, LANES))
            elif t[0] == 'B' and sb is not None:
                j = int(t[1:])
                p = jnp.exp2(sb[:, j * KB:(j + 1) * KB] - jnp.tile(st['m'], (1, KB // LANES)))
                ls = _lane_reduce(jnp.add, p)
                st['l'] = ls if 'l' not in st else st['l'] + ls
                o = jnp.dot(p.astype(jnp.bfloat16), v_ref[j * KB:(j + 1) * KB, :],
                            preferred_element_type=jnp.float32)
                st['o'] = o if 'o' not in st else st['o'] + o
            elif t == 'F' and sb is not None:
                l = jnp.sum(st['l'], axis=-1, keepdims=True)
                r = pl.reciprocal(l, approx=True)
                r = r * (2.0 - l * r)
                o_ref[...] = (st['o'] * r).astype(o_ref.dtype)

    FULL = "M A0 A1 A2 B0 B1 B2 B3 F A3"

    def in_copies(it, slot):
        h = N1 + it * U
        return [pltpu.make_async_copy(v_hbm.at[pl.ds(h, U)], vb.at[slot], sem_in.at[slot, 0]),
                pltpu.make_async_copy(k_hbm.at[pl.ds(h + 1, U)], kb.at[slot], sem_in.at[slot, 1]),
                pltpu.make_async_copy(q_hbm.at[pl.ds(h + 1, U)], qb.at[slot], sem_in.at[slot, 2])]

    def out_copy(it, slot):
        return pltpu.make_async_copy(ob.at[slot], o_hbm.at[pl.ds(N1 + it * U, U)], sem_out.at[slot])

    def pk(h): return pltpu.make_async_copy(k_hbm.at[h], kp.at[h], semp.at[h, 0])
    def pq(h): return pltpu.make_async_copy(q_hbm.at[h], qp.at[h], semp.at[h, 1])
    def pv(h): return pltpu.make_async_copy(v_hbm.at[h], vp.at[h], semp.at[h, 2])
    def po(h): return pltpu.make_async_copy(op.at[h], o_hbm.at[h], sempo.at[h])
    last_v = pltpu.make_async_copy(v_hbm.at[G - 1], vp.at[N1], semp.at[N1, 2])
    last_o = pltpu.make_async_copy(op.at[N1], o_hbm.at[G - 1], sempo.at[N1])

    def first_slot(u):
        h = N1 + u
        return [pltpu.make_async_copy(q_hbm.at[h + 1], qb.at[0, u], sem_s0.at[2, u]),
                pltpu.make_async_copy(k_hbm.at[h + 1], kb.at[0, u], sem_s0.at[0, u]),
                pltpu.make_async_copy(v_hbm.at[h], vb.at[0, u], sem_s0.at[1, u])]

    half = Sk // 2
    kc = [pltpu.make_async_copy(k_hbm.at[0, pl.ds(j * half, half)],
                                kp.at[0, pl.ds(j * half, half)], semk0.at[j]) for j in range(2)]

    pq(0).start(); kc[0].start(); kc[1].start()
    for h in range(N1):
        pq(h + 1).start(); pk(h + 1).start(); pv(h).start()
    pq(0).wait(); kc[0].wait()
    st0 = {}
    run("A0 A1", lambda j: qp.at[0], kp.at[0], S[0].at[0], M[0].at[0], None, None, None, None, st0)
    kc[1].wait()
    run("A2 A3", lambda j: qp.at[0], kp.at[0], S[0].at[0], M[0].at[0], None, None, None, None, st0)
    for h in range(N1):
        pq(h + 1).wait(); pk(h + 1).wait()
        args = (lambda j, h=h: qp.at[h + 1], kp.at[h + 1], S[(h + 1) % NS].at[0], M[(h + 1) % NS].at[0],
                S[h % NS].at[0], M[h % NS].at[0], vp.at[h], op.at[h])
        if h == 0:
            sth = {}
            run("M A0 A1 A2", *args, sth)
            pv(h).wait()
            run("B0 B1 B2 B3 F A3", *args, sth)
        else:
            pv(h).wait()
            if h == 2:
                for u in range(U):
                    for x in first_slot(u): x.start()
            run(FULL, *args)
        po(h).start()
    for kind in (1, 2, 0):
        for u in range(U): first_slot(u)[kind].wait()
    for x in in_copies(1, 1): x.start()
    last_v.start()

    def body(it, carry):
        slot = it & 1
        z1 = it >> 12
        z2 = (it + 1) >> 12

        @pl.when(it >= 2)
        def _():
            out_copy(it - 2, slot).wait()

        @pl.when(it >= 1)
        def _():
            for x in in_copies(it, slot): x.wait()

        for u in range(U):
            a, b = (N1 + u + 1) % NS, (N1 + u) % NS
            run(FULL, lambda j, u=u: qb.at[slot, u + ((it + j) >> 12)], kb.at[slot, u],
                S[a].at[z1], M[a].at[z1], S[b].at[z2], M[b].at[z2], vb.at[slot, u], ob.at[slot, u])
        out_copy(it, slot).start()

        @pl.when(it + 2 < NIT)
        def _():
            for x in in_copies(it + 2, slot): x.start()
        return carry

    lax.fori_loop(0, NIT, body, 0)

    last_v.wait()
    run(FULL, None, None, None, None, S[(G - 1) % NS].at[0], M[(G - 1) % NS].at[0], vp.at[N1], op.at[N1])
    last_o.start()
    out_copy(NIT - 2, (NIT - 2) % 2).wait()
    out_copy(NIT - 1, (NIT - 1) % 2).wait()
    for h in range(N1): po(h).wait()
    last_o.wait()


@jax.jit
def pallas_standalone__gqa_softmax__near_ridge_kernel(q, k, v):
    Bn, Hq, Sq, D = q.shape
    Hkv, Sk = k.shape[1], k.shape[2]
    G, R = Bn * Hkv, (Hq // Hkv) * Sq
    dt = q.dtype
    anyspec = pl.BlockSpec(memory_space=pl.ANY)
    dma = pltpu.SemaphoreType.DMA
    o = pl.pallas_call(
        _kernel, grid=(),
        in_specs=[anyspec] * 3, out_specs=anyspec,
        out_shape=jax.ShapeDtypeStruct((G, R, D), dt),
        scratch_shapes=[
            pltpu.VMEM((2, U, R, D), dt), pltpu.VMEM((2, U, Sk, D), dt),
            pltpu.VMEM((2, U, Sk, D), dt), pltpu.VMEM((2, U, R, D), dt),
            pltpu.VMEM((N1 + 1, R, D), dt), pltpu.VMEM((N1 + 1, Sk, D), dt),
            pltpu.VMEM((N1 + 1, Sk, D), dt), pltpu.VMEM((N1 + 1, R, D), dt),
            pltpu.VMEM((1, R, Sk), jnp.float32), pltpu.VMEM((1, R, Sk), jnp.float32),
            pltpu.VMEM((1, R, LANES), jnp.float32), pltpu.VMEM((1, R, LANES), jnp.float32),
            dma((2, 3)), dma((2,)), dma((N1 + 1, 3)), dma((N1 + 1,)), dma((3, U)), dma((2,)),
        ],
        compiler_params=pltpu.CompilerParams(
            vmem_limit_bytes=100 * 2**20,
            flags={"XLA_TPU_FORCE_LP_LLO_SCHEDULER": True}),
    )(q.reshape(G, R, D), k.reshape(G, Sk, D), v.reshape(G, Sk, D))
    return o.reshape(Bn, Hq, Sq, D)
```

```python
import jax
import jax.numpy as jnp
from jax import lax
from jax.experimental import pallas as pl
from jax.experimental.pallas import tpu as pltpu

LOG2E = 1.4426950408889634
U = 4
N1 = 7
NS = 2
KB = 512
LANES = 128


def _lane_reduce(op, s):
    r = s[:, :LANES]
    for t in range(1, s.shape[1] // LANES):
        r = op(r, s[:, t * LANES:(t + 1) * LANES])
    return r


def _kernel(q_hbm, k_hbm, v_hbm, o_hbm, qb, kb, vb, ob, qp, kp, vp, op,
            s0, s1, m0, m1, sem_in, sem_out, semp, sempo, sem_s0, semk0):
    S, M = (s0, s1), (m0, m1)
    G, R, D = q_hbm.shape
    Sk = k_hbm.shape[1]
    NB = Sk // KB
    c = D ** -0.5 * LOG2E
    assert NB == 4 and (G - 1 - N1) % U == 0 and G < 4000
    NIT = (G - 1 - N1) // U

    def run(toks, qf, k_ref, sa, ma, sb, mb, v_ref, o_ref, st=None):
        st = {} if st is None else st
        for t in toks.split():
            if t[0] == 'A' and qf is not None:
                j = int(t[1:])
                q = (qf(j)[...].astype(jnp.float32) * c).astype(jnp.bfloat16)
                s = lax.dot_general(q, k_ref[j * KB:(j + 1) * KB, :], (((1,), (1,)), ((), ())),
                                    preferred_element_type=jnp.float32)
                sa[:, j * KB:(j + 1) * KB] = s
                pm = _lane_reduce(jnp.maximum, s)
                st['pm'] = pm if 'pm' not in st else jnp.maximum(st['pm'], pm)
                if j == NB - 1:
                    ma[...] = st['pm']
            elif t == 'M' and sb is not None:
                st['m'] = jnp.broadcast_to(jnp.max(mb[...], axis=-1, keepdims=True), (R, LANES))
            elif t[0] == 'B' and sb is not None:
                j = int(t[1:])
                p = jnp.exp2(sb[:, j * KB:(j + 1) * KB] - jnp.tile(st['m'], (1, KB // LANES)))
                ls = _lane_reduce(jnp.add, p)
                st['l'] = ls if 'l' not in st else st['l'] + ls
                o = jnp.dot(p.astype(jnp.bfloat16), v_ref[j * KB:(j + 1) * KB, :],
                            preferred_element_type=jnp.float32)
                st['o'] = o if 'o' not in st else st['o'] + o
            elif t == 'F' and sb is not None:
                l = jnp.sum(st['l'], axis=-1, keepdims=True)
                r = pl.reciprocal(l, approx=True)
                r = r * (2.0 - l * r)
                o_ref[...] = (st['o'] * r).astype(o_ref.dtype)

    FULL = "M A0 A1 A2 B0 B1 B2 B3 F A3"

    def in_copies(it, slot):
        h = N1 + it * U
        return [pltpu.make_async_copy(v_hbm.at[pl.ds(h, U)], vb.at[slot], sem_in.at[slot, 0]),
                pltpu.make_async_copy(k_hbm.at[pl.ds(h + 1, U)], kb.at[slot], sem_in.at[slot, 1]),
                pltpu.make_async_copy(q_hbm.at[pl.ds(h + 1, U)], qb.at[slot], sem_in.at[slot, 2])]

    def out_copy(it, slot):
        return pltpu.make_async_copy(ob.at[slot], o_hbm.at[pl.ds(N1 + it * U, U)], sem_out.at[slot])

    def pk(h): return pltpu.make_async_copy(k_hbm.at[h], kp.at[h], semp.at[h, 0])
    def pq(h): return pltpu.make_async_copy(q_hbm.at[h], qp.at[h], semp.at[h, 1])
    def pv(h): return pltpu.make_async_copy(v_hbm.at[h], vp.at[h], semp.at[h, 2])
    def po(h): return pltpu.make_async_copy(op.at[h], o_hbm.at[h], sempo.at[h])
    last_v = pltpu.make_async_copy(v_hbm.at[G - 1], vp.at[N1], semp.at[N1, 2])
    last_o = pltpu.make_async_copy(op.at[N1], o_hbm.at[G - 1], sempo.at[N1])

    def first_slot(kind, u):
        h = N1 + u
        if kind == 0:
            return pltpu.make_async_copy(q_hbm.at[h + 1], qb.at[0, u], sem_s0.at[2, u])
        if kind == 1:
            return pltpu.make_async_copy(k_hbm.at[h + 1], kb.at[0, u], sem_s0.at[0, u])
        return pltpu.make_async_copy(v_hbm.at[h], vb.at[0, u], sem_s0.at[1, u])

    half = Sk // 2
    kc = [pltpu.make_async_copy(k_hbm.at[0, pl.ds(j * half, half)],
                                kp.at[0, pl.ds(j * half, half)], semk0.at[j]) for j in range(2)]

    pq(0).start(); kc[0].start(); kc[1].start()
    for h in range(N1):
        pq(h + 1).start(); pk(h + 1).start(); pv(h).start()
    pq(0).wait(); kc[0].wait()
    st0 = {}
    run("A0 A1", lambda j: qp.at[0], kp.at[0], S[0].at[0], M[0].at[0], None, None, None, None, st0)
    kc[1].wait()
    run("A2 A3", lambda j: qp.at[0], kp.at[0], S[0].at[0], M[0].at[0], None, None, None, None, st0)
    for h in range(N1):
        pq(h + 1).wait(); pk(h + 1).wait()
        args = (lambda j, h=h: qp.at[h + 1], kp.at[h + 1], S[(h + 1) % NS].at[0], M[(h + 1) % NS].at[0],
                S[h % NS].at[0], M[h % NS].at[0], vp.at[h], op.at[h])
        if h == 0:
            sth = {}
            run("M A0 A1 A2", *args, sth)
            pv(h).wait()
            run("B0 B1 B2 B3 F A3", *args, sth)
        else:
            pv(h).wait()
            if h == 2:
                for u in range(U):
                    for kind in range(3): first_slot(kind, u).start()
            run(FULL, *args)
        po(h).start()
    for kind in (1, 2, 0):
        for u in range(U): first_slot(kind, u).wait()
    for x in in_copies(1, 1): x.start()
    last_v.start()

    def body(it, carry):
        slot = it & 1
        z1 = it >> 12
        z2 = (it + 1) >> 12

        @pl.when(it >= 2)
        def _():
            out_copy(it - 2, slot).wait()

        @pl.when(it >= 1)
        def _():
            for x in in_copies(it, slot): x.wait()

        for u in range(U):
            a, b = (N1 + u + 1) % NS, (N1 + u) % NS
            run(FULL, lambda j, u=u: qb.at[slot, u + ((it + j) >> 12)], kb.at[slot, u],
                S[a].at[z1], M[a].at[z1], S[b].at[z2], M[b].at[z2], vb.at[slot, u], ob.at[slot, u])
        out_copy(it, slot).start()

        @pl.when(it + 2 < NIT)
        def _():
            for x in in_copies(it + 2, slot): x.start()
        return carry

    lax.fori_loop(0, NIT, body, 0)

    last_v.wait()
    run(FULL, None, None, None, None, S[(G - 1) % NS].at[0], M[(G - 1) % NS].at[0], vp.at[N1], op.at[N1])
    last_o.start()
    out_copy(NIT - 2, (NIT - 2) % 2).wait()
    out_copy(NIT - 1, (NIT - 1) % 2).wait()
    for h in range(N1): po(h).wait()
    last_o.wait()


@jax.jit
def pallas_standalone__gqa_softmax__near_ridge_kernel(q, k, v):
    Bn, Hq, Sq, D = q.shape
    Hkv, Sk = k.shape[1], k.shape[2]
    G, R = Bn * Hkv, (Hq // Hkv) * Sq
    dt = q.dtype
    anyspec = pl.BlockSpec(memory_space=pl.ANY)
    dma = pltpu.SemaphoreType.DMA
    o = pl.pallas_call(
        _kernel, grid=(),
        in_specs=[anyspec] * 3, out_specs=anyspec,
        out_shape=jax.ShapeDtypeStruct((G, R, D), dt),
        scratch_shapes=[
            pltpu.VMEM((2, U, R, D), dt), pltpu.VMEM((2, U, Sk, D), dt),
            pltpu.VMEM((2, U, Sk, D), dt), pltpu.VMEM((2, U, R, D), dt),
            pltpu.VMEM((N1 + 1, R, D), dt), pltpu.VMEM((N1 + 1, Sk, D), dt),
            pltpu.VMEM((N1 + 1, Sk, D), dt), pltpu.VMEM((N1 + 1, R, D), dt),
            pltpu.VMEM((1, R, Sk), jnp.float32), pltpu.VMEM((1, R, Sk), jnp.float32),
            pltpu.VMEM((1, R, LANES), jnp.float32), pltpu.VMEM((1, R, LANES), jnp.float32),
            dma((2, 3)), dma((2,)), dma((N1 + 1, 3)), dma((N1 + 1,)), dma((3, U)), dma((2,)),
        ],
        compiler_params=pltpu.CompilerParams(
            vmem_limit_bytes=100 * 2**20,
            flags={"XLA_TPU_FORCE_LP_LLO_SCHEDULER": True}),
    )(q.reshape(G, R, D), k.reshape(G, Sk, D), v.reshape(G, Sk, D))
    return o.reshape(Bn, Hq, Sq, D)
```
